```python
import jax
import jax.numpy as jnp

def _softmax(x, axis=-1):
    return jax.nn.softmax(x, axis=axis)
def _gelu(x):
    return jax.nn.gelu(x, approximate=True)
def _silu(x):
    return jax.nn.silu(x)
def _sigmoid(x):
    return jax.nn.sigmoid(x)
def _layernorm(x, axis=-1, eps=1e-5):
    m = jnp.mean(x, axis=axis, keepdims=True)
    v = jnp.var(x, axis=axis, keepdims=True)
    return (x - m) / jnp.sqrt(v + eps)
def _scatter_add(tgt, idx, src, axis=0):
    return tgt.at[idx].add(src)
def _segment_sum(src, seg, n):
    return jax.ops.segment_sum(src, seg, n)
class _Rng:
    def __init__(self, key):
        self._k = key
    def _next(self):
        self._k, sub = jax.random.split(self._k)
        return sub
    def normal(self, shape):
        return jax.random.normal(self._next(), shape, dtype=jnp.bfloat16)
    def randint(self, lo, hi, shape):
        return jax.random.randint(self._next(), shape, lo, hi, dtype=jnp.int32)
    def uniform(self, shape, lo=0.0, hi=1.0):
        return jax.random.uniform(self._next(), shape, jnp.bfloat16, lo, hi)
    def permutation(self, n):
        return jax.random.permutation(self._next(), n)


kernel_name = 'concat_heads__gqa_block_cached__gqa_block_cached__near_ridge'

def setup_inputs():
    _rng = _Rng(jax.random.key(int.from_bytes(__import__("os").urandom(4), "little")))
    _w = (lambda a: (lambda t: t.astype(jnp.bfloat16) if jnp.issubdtype(t.dtype, jnp.floating) else t)(jnp.asarray(a)))
    def _A_setup():
        B, Sq, D = 8, 256, 640
        Hq, Hkv, Sk, Dh = 32, 32, 1024, 192
        assert Hq % Hkv == 0, (Hq, Hkv)
        return {
            "x": _w((lambda *s: _rng.normal(s) * 0.05)(B, Sq, D)),
            "k_cache": _w((lambda *s: _rng.normal(s) * 0.05)(B, Hkv, Sk, Dh)),
            "v_cache": _w((lambda *s: _rng.normal(s) * 0.05)(B, Hkv, Sk, Dh)),
            "wq": _w((lambda *s: _rng.normal(s) * 0.05)(D, Hq * Dh) * (D ** -0.5)),
            "wo": _w((lambda *s: _rng.normal(s) * 0.05)(Hq * Dh, D) * ((Hq * Dh) ** -0.5)),
        }
    _A_in = _A_setup()

    def _B_setup():
        B, Sq, D = 8, 256, 640
        Hq, Hkv, Sk, Dh = 32, 32, 1024, 192
        assert Hq % Hkv == 0, (Hq, Hkv)
        return {
            "x": _w((lambda *s: _rng.normal(s) * 0.05)(B, Sq, D)),
            "k_cache": _w((lambda *s: _rng.normal(s) * 0.05)(B, Hkv, Sk, Dh)),
            "v_cache": _w((lambda *s: _rng.normal(s) * 0.05)(B, Hkv, Sk, Dh)),
            "wq": _w((lambda *s: _rng.normal(s) * 0.05)(D, Hq * Dh) * (D ** -0.5)),
            "wo": _w((lambda *s: _rng.normal(s) * 0.05)(Hq * Dh, D) * ((Hq * Dh) ** -0.5)),
        }
    _B_in = _B_setup()

    return {
        "A_x": _A_in["x"],
        "A_k_cache": _A_in["k_cache"],
        "A_v_cache": _A_in["v_cache"],
        "A_wq": _A_in["wq"],
        "A_wo": _A_in["wo"],
        "B_x": _B_in["x"],
        "B_k_cache": _B_in["k_cache"],
        "B_v_cache": _B_in["v_cache"],
        "B_wq": _B_in["wq"],
        "B_wo": _B_in["wo"],
    }

def reference(A_x, A_k_cache, A_v_cache, A_wq, A_wo, B_x, B_k_cache, B_v_cache, B_wq, B_wo):
    def _A_ref(x, k_cache, v_cache, wq, wo):
        B, Sq, D = x.shape
        Hq, Dh = 32, 192
        Hkv = k_cache.shape[1]
        rep = Hq // Hkv
        q = (lambda x, *d: x.transpose(*d))((x @ wq).reshape(B, Sq, Hq, Dh), 0, 2, 1, 3)
        k = jnp.repeat(k_cache, rep, axis=1)
        v = jnp.repeat(v_cache, rep, axis=1)
        scores = jnp.einsum("bhqd,bhkd->bhqk", q, k) * (Dh ** -0.5)
        p = _softmax(scores, axis=-1)
        o = jnp.einsum("bhqk,bhkd->bhqd", p, v)
        return (lambda x, *d: x.transpose(*d))(o, 0, 2, 1, 3).reshape(B, Sq, Hq * Dh) @ wo

    def _B_ref(x, k_cache, v_cache, wq, wo):
        B, Sq, D = x.shape
        Hq, Dh = 32, 192
        Hkv = k_cache.shape[1]
        rep = Hq // Hkv
        q = (lambda x, *d: x.transpose(*d))((x @ wq).reshape(B, Sq, Hq, Dh), 0, 2, 1, 3)
        k = jnp.repeat(k_cache, rep, axis=1)
        v = jnp.repeat(v_cache, rep, axis=1)
        scores = jnp.einsum("bhqd,bhkd->bhqk", q, k) * (Dh ** -0.5)
        p = _softmax(scores, axis=-1)
        o = jnp.einsum("bhqk,bhkd->bhqd", p, v)
        return (lambda x, *d: x.transpose(*d))(o, 0, 2, 1, 3).reshape(B, Sq, Hq * Dh) @ wo

    a = _A_ref(A_x, A_k_cache, A_v_cache, A_wq, A_wo)
    b = _B_ref(B_x, B_k_cache, B_v_cache, B_wq, B_wo)
    return jnp.concatenate([a, b], axis=-1)
```

```python
import functools
import jax
import jax.numpy as jnp
import jax.experimental.pallas as pl
import jax.experimental.pallas.tpu as pltpu

DH = 192
LOG2E = 1.4426950408889634
NT = ((1,), (1,)), ((), ())
PW = 2 * DH


def qproj(x, wq):
    c = (DH ** -0.5) * LOG2E
    q = jnp.dot(x, wq, preferred_element_type=jnp.float32) * c
    qb = q.astype(jnp.bfloat16)
    lane = jax.lax.broadcasted_iota(jnp.int32, (q.shape[0], 128), 1)
    mid = qb[:, 128:256]
    zero = jnp.zeros_like(mid)
    q0 = jnp.concatenate([qb[:, 0:128], jnp.where(lane < 64, mid, zero)], axis=1)
    q1 = jnp.concatenate([jnp.where(lane >= 64, mid, zero), qb[:, 256:384]], axis=1)
    return q0, q1


class Head:
    def __init__(self, q, kt_ref, vt_ref, h, CW):
        self.q, self.kt_ref, self.vt_ref, self.h, self.CW = q, kt_ref, vt_ref, h, CW
        self.s = []
        self.pm = None
        self.pl = None
        self.ot = None

    def qk(self, j):
        CW = self.CW
        r0 = self.h * 128
        kt = self.kt_ref[r0:r0 + 256, j * CW:(j + 1) * CW]
        s = jnp.dot(self.q, kt, preferred_element_type=jnp.float32)
        self.s.append(s)
        pm = s[:, 0:128]
        for t in range(1, CW // 128):
            pm = jnp.maximum(pm, s[:, t * 128:(t + 1) * 128])
        self.pm = pm if self.pm is None else jnp.maximum(self.pm, pm)

    def mx(self):
        self.m = jnp.max(self.pm, axis=-1, keepdims=True)

    def ex(self, j):
        CW = self.CW
        p = jnp.exp2(self.s[j] - self.m)
        ps = p[:, 0:128]
        for t in range(1, CW // 128):
            ps = ps + p[:, t * 128:(t + 1) * 128]
        self.pl = ps if self.pl is None else self.pl + ps
        self.p = p.astype(jnp.bfloat16)

    def pv(self, j):
        CW = self.CW
        r0 = self.h * DH
        vt = self.vt_ref[r0:r0 + DH, j * CW:(j + 1) * CW]
        o = jax.lax.dot_general(vt, self.p, NT, preferred_element_type=jnp.float32)
        self.ot = o if self.ot is None else self.ot + o

    def fin(self):
        self.r = 1.0 / jnp.sum(self.pl, axis=-1, keepdims=True)


def oprep(h0, h1):
    ot = jnp.concatenate([h0.ot, h1.ot], axis=0)
    return oprep2(ot, h0.r, h1.r)


def oprep2(ot, r0, r1):
    o = ot.T
    lane3 = jax.lax.broadcasted_iota(jnp.int32, o.shape, 1)
    r = jnp.where(lane3 < DH, r0, r1)
    return (o * r).astype(jnp.bfloat16)


def make(NP, CW=256, OPAR=1, QJ=3, **kw):
    HGW = NP * PW

    def kernel(xa, ka, va, wqa, woa, xb, kb, vb, wqb, wob, o_hbm,
               xs, wqs, wos, ks, vs, acc_ref, ob, qc, oc, rc, xsem, wsem, kvsem, osem):
        NB = xa.shape[0]
        NHG = ka.shape[1] // HGW
        NC = 1024 // CW
        xh, kh, vh, wqh, woh = (xa, xb), (ka, kb), (va, vb), (wqa, wqb), (woa, wob)

        def x_copy(br, b):
            return pltpu.make_async_copy(xh[br].at[b], xs.at[br, b], xsem.at[br, b])

        def wq_copy(br, hg):
            c = pl.ds(pl.multiple_of(hg * HGW, 128), HGW)
            return pltpu.make_async_copy(wqh[br].at[:, c], wqs.at[br, hg], wsem.at[0, br, hg % 2])

        def wo_copy(br, hg):
            c = pl.ds(pl.multiple_of(hg * HGW, 128), HGW)
            return pltpu.make_async_copy(woh[br].at[c, :], wos.at[br, hg], wsem.at[1, br, hg % 2])

        def kv_copy(which, i, hg, b, par):
            br, p = i % 2, i // 2
            c = pl.ds(pl.multiple_of(hg * HGW + p * PW, PW), PW)
            src = (kh, vh)[which][br].at[b, c, :]
            dst = (ks, vs)[which].at[par, i]
            return pltpu.make_async_copy(src, dst, kvsem.at[which, par, i])

        def o_copy(b):
            return pltpu.make_async_copy(ob.at[b], o_hbm.at[b], osem.at[b])

        x_copy(0, 0).start(); wq_copy(0, 0).start(); kv_copy(0, 0, 0, 0, 0).start()
        x_copy(1, 0).start(); wq_copy(1, 0).start(); kv_copy(1, 0, 0, 0, 0).start()
        for i in range(1, 2 * NP):
            kv_copy(0, i, 0, 0, 0).start()
            if i == 1:
                wo_copy(0, 0).start(); wo_copy(1, 0).start()
            kv_copy(1, i, 0, 0, 0).start()

        NT_ = NHG * NB
        LP = 2 * NP - 1
        acc_ref[...] = jnp.zeros(acc_ref.shape, jnp.float32)
        oc[...] = jnp.zeros(oc.shape, oc.dtype)
        rc[...] = jnp.ones(rc.shape, rc.dtype)
        def ocarry():
            return oprep2(oc[...], 1.0 / jnp.sum(rc[0], axis=-1, keepdims=True), 1.0 / jnp.sum(rc[1], axis=-1, keepdims=True))
        x_copy(0, 1).start()
        x_copy(0, 0).wait(); wq_copy(0, 0).wait()
        if NHG > 1:
            wq_copy(0, 1).start()

        def q_to_carry(hg, b):
            q0, q1 = qproj(xs[0, b], wqs[0, hg, :, 0:PW])
            qc[0] = q0
            qc[1] = q1

        q_to_carry(0, 0)
        chunks = [(0, 128), (128, 256), (256, 384), (384, 640)]

        def oproj(o, i, hg, b, lo, hi):
            br, p = i % 2, i // 2
            off = br * 640
            acc_ref[b, :, off + lo:off + hi] += jnp.dot(
                o, wos[br, hg, p * PW:(p + 1) * PW, lo:hi], preferred_element_type=jnp.float32)

        def body(t, _):
            hg, b = t // NB, t % NB
            par = t % 2
            tn = jnp.minimum(t + 1, NT_ - 1)
            hgn, bn = tn // NB, tn % NB
            tp = jnp.maximum(t - 1, 0)
            hgp, bp = tp // NB, tp % NB

            @pl.when(b == 0)
            def _():
                wq_copy(1, hg).wait()
                wo_copy(0, hg).wait(); wo_copy(1, hg).wait()
                @pl.when(hg + 1 < NHG)
                def _():
                    wq_copy(1, hg + 1).start()
                    for br in range(2):
                        wo_copy(br, hg + 1).start()

            @pl.when(jnp.logical_and(b == NB - 1, hg + 1 < NHG))
            def _():
                wq_copy(0, hg + 1).wait()
                @pl.when(hg + 2 < NHG)
                def _():
                    wq_copy(0, hg + 2).start()

            @pl.when(hg == 0)
            def _():
                x_copy(1, b).wait()
                @pl.when(b + 1 < NB)
                def _():
                    x_copy(0, b + 1).wait()
                    x_copy(1, b + 1).start()
                @pl.when(b + 2 < NB)
                def _():
                    x_copy(0, b + 2).start()

            for i in range(2 * NP):
                kv_copy(0, i, hg, b, par).wait()
                kv_copy(1, i, hg, b, par).wait()

            def mkheads(i):
                br, p = i % 2, i // 2
                if i == 0:
                    q0, q1 = qc[0], qc[1]
                else:
                    q0, q1 = qproj(xs[br, b], wqs[br, hg, :, p * PW:(p + 1) * PW])
                return [Head(q0, ks.at[par, i], vs.at[par, i], 0, CW),
                        Head(q1, ks.at[par, i], vs.at[par, i], 1, CW)]

            heads = mkheads(0)
            for j in range(NC):
                heads[0].qk(j)
            heads[0].mx()
            for i in range(2 * NP):
                kv_copy(0, i, hgn, bn, 1 - par).start()
                kv_copy(1, i, hgn, bn, 1 - par).start()
            nh = 4 * NP
            pending = functools.partial(oproj, ocarry(), LP, hgp, bp)
            for i in range(nh):
                if i % 2 == 0 and i + 2 < nh:
                    heads += mkheads(i // 2 + 1)
                for j in range(NC):
                    heads[i].ex(j)
                    if i + 1 < nh:
                        heads[i + 1].qk(j)
                    if i % 2 == OPAR:
                        [pending(*chunks[c]) for c in range(j * 4 // NC, (j + 1) * 4 // NC)]
                    heads[i].pv(j)
                    if i == nh - 1 and j == min(QJ, NC - 1):
                        q_to_carry(hgn, bn)
                heads[i].fin()
                if i + 1 < nh:
                    heads[i + 1].mx()
                if i % 2 == 1:
                    if i == nh - 1:
                        oc[0:DH] = heads[i - 1].ot
                        oc[DH:PW] = heads[i].ot
                        rc[0] = heads[i - 1].pl
                        rc[1] = heads[i].pl
                    else:
                        o = oprep(heads[i - 1], heads[i])
                        pending = functools.partial(oproj, o, i // 2, hg, b)

            @pl.when(jnp.logical_and(hgp == NHG - 1, t > 0))
            def _():
                ob[bp] = acc_ref[bp].astype(ob.dtype)
                o_copy(bp).start()
            return None

        jax.lax.fori_loop(0, NT_, body, None)
        olast = ocarry()
        for lo, hi in chunks:
            oproj(olast, LP, NHG - 1, NB - 1, lo, hi)
        ob[NB - 1] = acc_ref[NB - 1].astype(ob.dtype)
        o_copy(NB - 1).start()
        for i in range(2 * NP):
            kv_copy(0, i, NHG - 1, NB - 1, (NHG * NB) % 2).wait()
            kv_copy(1, i, NHG - 1, NB - 1, (NHG * NB) % 2).wait()
        for b in range(NB):
            o_copy(b).wait()

    def fn(A_x, A_k_cache, A_v_cache, A_wq, A_wo, B_x, B_k_cache, B_v_cache, B_wq, B_wo):
        B, Sq, D = A_x.shape
        _, H, Sk, Dh = A_k_cache.shape
        NHG = H // 2 // NP

        def tr(c):
            return jnp.transpose(c, (0, 1, 3, 2)).reshape(B, H * Dh, Sk)

        any_spec = pl.BlockSpec(memory_space=pl.ANY)
        return pl.pallas_call(
            kernel,
            in_specs=[any_spec] * 10,
            out_specs=any_spec,
            out_shape=jax.ShapeDtypeStruct((B, Sq, 2 * D), jnp.bfloat16),
            scratch_shapes=[
                pltpu.VMEM((2, B, Sq, D), jnp.bfloat16),
                pltpu.VMEM((2, NHG, D, HGW), jnp.bfloat16),
                pltpu.VMEM((2, NHG, HGW, D), jnp.bfloat16),
                pltpu.VMEM((2, 2 * NP, PW, Sk), jnp.bfloat16),
                pltpu.VMEM((2, 2 * NP, PW, Sk), jnp.bfloat16),
                pltpu.VMEM((B, Sq, 2 * D), jnp.float32),
                pltpu.VMEM((B, Sq, 2 * D), jnp.bfloat16),
                pltpu.VMEM((2, Sq, 256), jnp.bfloat16),
                pltpu.VMEM((PW, Sq), jnp.float32),
                pltpu.VMEM((2, Sq, 128), jnp.float32),
                pltpu.SemaphoreType.DMA((2, B)),
                pltpu.SemaphoreType.DMA((2, 2, 2)),
                pltpu.SemaphoreType.DMA((2, 2, 2 * NP)),
                pltpu.SemaphoreType.DMA((B,)),
            ],
            compiler_params=pltpu.CompilerParams(vmem_limit_bytes=110 * 1024 * 1024, **kw),
        )(A_x, tr(A_k_cache), tr(A_v_cache), A_wq, A_wo,
          B_x, tr(B_k_cache), tr(B_v_cache), B_wq, B_wo)
    return fn


_impl = make(2, 256, 1, 2, disable_bounds_checks=True)


@jax.jit
def pallas_concat_heads__gqa_block_cached__gqa_block_cached__near_ridge_kernel(
    A_x, A_k_cache, A_v_cache, A_wq, A_wo, B_x, B_k_cache, B_v_cache, B_wq, B_wo
):
    return _impl(A_x, A_k_cache, A_v_cache, A_wq, A_wo,
                 B_x, B_k_cache, B_v_cache, B_wq, B_wo)
```
